```python
import os as _os
_os.environ.setdefault("JAX_PLATFORMS", "cpu")
import jax
import jax.numpy as jnp

def _softmax(x, axis=-1):
    return jax.nn.softmax(x, axis=axis)
def _gelu(x):
    return jax.nn.gelu(x, approximate=True)
def _silu(x):
    return jax.nn.silu(x)
def _sigmoid(x):
    return jax.nn.sigmoid(x)
def _layernorm(x, axis=-1, eps=1e-5):
    m = jnp.mean(x, axis=axis, keepdims=True)
    v = jnp.var(x, axis=axis, keepdims=True)
    return (x - m) / jnp.sqrt(v + eps)
def _scatter_add(tgt, idx, src, axis=0):
    return tgt.at[idx].add(src)
def _segment_sum(src, seg, n):
    return jax.ops.segment_sum(src, seg, n)
class _Rng:
    def __init__(self, key):
        self._k = key
    def _next(self):
        self._k, sub = jax.random.split(self._k)
        return sub
    def normal(self, shape):
        return jax.random.normal(self._next(), shape, dtype=jnp.bfloat16)
    def randint(self, lo, hi, shape):
        return jax.random.randint(self._next(), shape, lo, hi, dtype=jnp.int32)
    def uniform(self, shape, lo=0.0, hi=1.0):
        return jax.random.uniform(self._next(), shape, jnp.bfloat16, lo, hi)
    def permutation(self, n):
        return jax.random.permutation(self._next(), n)


kernel_name = 'interleave_layers__linear_kernel_hedgehog__dense_activation_silu__prompt'

def setup_inputs():
    _rng = _Rng(jax.random.key(int.from_bytes(__import__("os").urandom(4), "little")))
    _w = (lambda a: (lambda t: t.astype(jnp.bfloat16) if jnp.issubdtype(t.dtype, jnp.floating) else t)(jnp.asarray(a)))
    def _A_setup():
        B, S, D, H = 1, 2048, 640, 32
        Dh = D // H
        return {
            "x": _w((lambda *s: _rng.normal(s) * 0.05)(B, S, D)),
            "wqkv": _w((lambda *s: _rng.normal(s) * 0.4)(D, 3 * D)),
            "w_phi": _w((lambda *s: _rng.normal(s) * 0.4)(H, Dh, Dh) * (Dh ** -0.5)),
            "wo": _w((lambda *s: _rng.normal(s) * 0.05)(D, D)),
        }
    _A_in = _A_setup()

    def _B_setup():
        B, S, D, F = 1, 2048, 640, 1728
        return {
            "x": _w((lambda *s: _rng.normal(s) * 0.05)(B, S, D)),
            "w1": _w((lambda *s: _rng.normal(s) * 1.6)(D, F) * (D ** -0.5)),
            "w2": _w((lambda *s: _rng.normal(s) * 1.6)(F, D) * (F ** -0.5)),
        }
    _B_in = _B_setup()

    return {
        "A_x": _A_in["x"],
        "A_wqkv": _A_in["wqkv"],
        "A_w_phi": _A_in["w_phi"],
        "A_wo": _A_in["wo"],
        "B_x": _B_in["x"],
        "B_w1": _B_in["w1"],
        "B_w2": _B_in["w2"],
    }

def reference(A_x, A_wqkv, A_w_phi, A_wo, B_x, B_w1, B_w2):
    def _A_ref(x, wqkv, w_phi, wo):
        B, S, D = x.shape
        H = 32; Dh = D // H
        qkv = (lambda x, *d: x.transpose(*d))((x @ wqkv).reshape(B, S, 3, H, Dh), 2, 0, 3, 1, 4)
        q, k, v = qkv[0], qkv[1], qkv[2]
        pq = jnp.einsum("bhsd,hdf->bhsf", q, w_phi)
        pk = jnp.einsum("bhsd,hdf->bhsf", k, w_phi)
        phi_q = jnp.concatenate([_softmax(pq, axis=-1), _softmax(-pq, axis=-1)], axis=-1)
        phi_k = jnp.concatenate([_softmax(pk, axis=-1), _softmax(-pk, axis=-1)], axis=-1)
        kv = jnp.einsum("bhsf,bhsd->bhfd", phi_k, v)
        z  = jnp.einsum("bhsf->bhf", phi_k)
        num = jnp.einsum("bhqf,bhfd->bhqd", phi_q, kv)
        den = jnp.einsum("bhqf,bhf->bhq", phi_q, z)[..., None] + 1e-6
        o = num / den
        return (lambda x, *d: x.transpose(*d))(o, 0, 2, 1, 3).reshape(B, S, D) @ wo

    def _B_ref(x, w1, w2):
        h = jnp.einsum("bsd,df->bsf", x, w1)
        h = _silu(h)
        out = jnp.einsum("bsf,fd->bsd", h, w2)
        return out

    x = A_x
    x = x + _A_ref(_layernorm(x, axis=-1), A_wqkv, A_w_phi, A_wo)
    x = x + _B_ref(_layernorm(x, axis=-1), B_w1, B_w2)
    x = x + _A_ref(_layernorm(x, axis=-1), A_wqkv, A_w_phi, A_wo)
    x = x + _B_ref(_layernorm(x, axis=-1), B_w1, B_w2)
    return x
```

```python
import jax
import jax.numpy as jnp
from jax import lax
import jax.experimental.pallas as pl
import jax.experimental.pallas.tpu as pltpu

S = 2048
D = 640
H = 32
DH = 20
FF = 1728
HG = 2
LG = 1
NG = H // HG
GR = HG * DH
NV = GR // 8
TS = 512
NT = S // TS

_BF = jnp.bfloat16
_F32 = jnp.float32


def _dot_nn(a, b):
    return lax.dot_general(a, b, (((1,), (0,)), ((), ())), preferred_element_type=_F32)


def _dot_nt(a, b):
    return lax.dot_general(a, b, (((1,), (1,)), ((), ())), preferred_element_type=_F32)


def _dot_tn(a, b):
    return lax.dot_general(a, b, (((0,), (0,)), ((), ())), preferred_element_type=_F32)


def _layernorm(x):
    m = jnp.mean(x, axis=-1, keepdims=True)
    xc = x - m
    v = jnp.mean(xc * xc, axis=-1, keepdims=True)
    return xc / jnp.sqrt(v + 1e-5)


def _head_reduce(x, op, op2):
    r = op(x, axis=0)
    r = op2(r, pltpu.roll(r, 4, 0))
    r = op2(pltpu.roll(r, 2, 0), r)
    return r[None]


def _head_sum(x):
    return _head_reduce(x, jnp.sum, jnp.add)


def _dual_softmax(p):
    mx = _head_reduce(p, jnp.max, jnp.maximum)
    mn = _head_reduce(p, jnp.min, jnp.minimum)
    ea = jnp.exp(p - mx)
    eb = jnp.exp(mn - p)
    return ea / _head_sum(ea), eb / _head_sum(eb)


def _kernel(x_hbm, wqkv_hbm, wphi_hbm, wo_hbm, w1t_hbm, w2_hbm, o_hbm,
            x_ref, wqkv_ref, wphi_ref, wo_ref, w1t_ref, w2_ref, ostage_ref,
            xres_ref, xn_ref, wallt_ref, kv_ref, z_ref, kvb_ref, zc_ref,
            in_sems, out_sems, x_sems):
    cp_phi = pltpu.make_async_copy(wphi_hbm, wphi_ref, in_sems.at[0])
    cp_wq = pltpu.make_async_copy(wqkv_hbm.at[:, 0:D], wqkv_ref.at[:, 0:D], in_sems.at[1])
    cp_wk = pltpu.make_async_copy(wqkv_hbm.at[:, D:2 * D], wqkv_ref.at[:, D:2 * D], in_sems.at[2])
    cp_wv = pltpu.make_async_copy(wqkv_hbm.at[:, 2 * D:3 * D], wqkv_ref.at[:, 2 * D:3 * D], in_sems.at[3])
    cp_x = [pltpu.make_async_copy(x_hbm.at[t * TS:(t + 1) * TS, :], x_ref.at[t * TS:(t + 1) * TS, :],
                                  x_sems.at[t]) for t in range(NT)]
    cp_wo = pltpu.make_async_copy(wo_hbm, wo_ref, in_sems.at[4])
    cp_w1 = pltpu.make_async_copy(w1t_hbm, w1t_ref, in_sems.at[5])
    cp_w2 = pltpu.make_async_copy(w2_hbm, w2_ref, in_sems.at[6])
    for cp in [cp_phi, cp_wq, cp_wk, cp_wv] + cp_x + [cp_wo, cp_w1, cp_w2]:
        cp.start()

    rr = lax.broadcasted_iota(jnp.int32, (GR, DH), 0)
    fcol = lax.broadcasted_iota(jnp.int32, (GR, DH), 1)
    sel = ((rr >> LG) == fcol).astype(_BF)
    r2 = lax.broadcasted_iota(jnp.int32, (GR, GR), 0)
    c2 = lax.broadcasted_iota(jnp.int32, (GR, GR), 1)
    jr = r2 & (HG - 1)
    amask = (c2 >= jr * DH) & (c2 < jr * DH + DH)
    kr = lax.broadcasted_iota(jnp.int32, (GR, 2 * GR), 0)
    kc = lax.broadcasted_iota(jnp.int32, (GR, 2 * GR), 1)
    jj = kc & (HG - 1)
    kvmask = (kr >= jj * DH) & (kr < jj * DH + DH)

    cp_phi.wait()
    a_blk = []
    for gi in range(NG):
        a_full = _dot_nt(sel, wphi_ref[gi * GR:(gi + 1) * GR, :])
        a_blk.append(jnp.where(amask, a_full, 0.0).astype(_BF))
    cp_wq.wait()
    for gi in range(NG):
        wallt_ref[gi * GR:(gi + 1) * GR, :] = _dot_nt(
            a_blk[gi], wqkv_ref[:, gi * GR:(gi + 1) * GR]).astype(_BF)
    cp_wk.wait()
    for gi in range(NG):
        wallt_ref[D + gi * GR:D + (gi + 1) * GR, :] = _dot_nt(
            a_blk[gi], wqkv_ref[:, D + gi * GR:D + (gi + 1) * GR]).astype(_BF)
    cp_wv.wait()
    wallt_ref[2 * D:3 * D, :] = wqkv_ref[:, 2 * D:3 * D].T

    def layer(li, carry):
        kv_ref[...] = jnp.zeros(kv_ref.shape, _F32)
        z_ref[...] = jnp.zeros(z_ref.shape, _F32)

        def phase1(t, c):
            row = pl.multiple_of(t * TS, TS)

            @pl.when(li == 0)
            def _():
                pltpu.make_async_copy(x_hbm.at[pl.ds(row, TS), :], x_ref.at[pl.ds(row, TS), :],
                                      x_sems.at[t]).wait()
                xres_ref[pl.ds(row, TS), :] = x_ref[pl.ds(row, TS), :].astype(_F32)

            xn = _layernorm(xres_ref[pl.ds(row, TS), :]).astype(_BF)
            xn_ref[pl.ds(row, TS), :] = xn
            pt = _dot_nt(wallt_ref[D:3 * D, :], xn)
            for gi in range(NG):
                pk = pt[gi * GR:(gi + 1) * GR].reshape(NV, 8, TS)
                pa, pb = _dual_softmax(pk)
                phi = jnp.concatenate([pa.reshape(GR, TS), pb.reshape(GR, TS)], axis=0)
                vt = pt[D + gi * GR:D + (gi + 1) * GR].astype(_BF)
                kv_ref[gi] += _dot_nt(vt, phi.astype(_BF))
                zp = phi[:, 0:128]
                for i in range(1, TS // 128):
                    zp = zp + phi[:, i * 128:(i + 1) * 128]
                z_ref[gi] += zp
            return c

        lax.fori_loop(0, NT, phase1, 0)

        for gi in range(NG):
            kvb_ref[gi] = jnp.where(kvmask, kv_ref[gi], 0.0).astype(_BF)
            zc = jnp.sum(z_ref[gi], axis=1, keepdims=True)
            zc_ref[gi] = jnp.broadcast_to(zc, (2 * GR, 128))

        @pl.when(li == 0)
        def _():
            cp_wo.wait()
            cp_w1.wait()
            cp_w2.wait()

        def phase2(t, c):
            row = pl.multiple_of(t * TS, TS)
            pq = _dot_nt(wallt_ref[0:D, :], xn_ref[pl.ds(row, TS), :])
            ots = []
            for gi in range(NG):
                p = pq[gi * GR:(gi + 1) * GR].reshape(NV, 8, TS)
                pa, pb = _dual_softmax(p)
                zc = zc_ref[gi][:, 0:1]
                za = zc[0:GR].reshape(NV, 8, 1)
                zb = zc[GR:2 * GR].reshape(NV, 8, 1)
                den = _head_sum(pa * za) + _head_sum(pb * zb) + 1e-6
                inv = 1.0 / den
                phi = jnp.concatenate([(pa * inv).reshape(GR, TS), (pb * inv).reshape(GR, TS)], axis=0)
                ots.append(_dot_nn(kvb_ref[gi], phi.astype(_BF)))
            ot = jnp.concatenate(ots, axis=0).astype(_BF)
            att = _dot_tn(ot, wo_ref[...])
            x1 = xres_ref[pl.ds(row, TS), :] + att
            xn2 = _layernorm(x1).astype(_BF)
            h = _dot_nt(xn2, w1t_ref[...])
            h = h * (1.0 / (1.0 + jnp.exp(-h)))
            y = _dot_nn(h.astype(_BF), w2_ref[...])
            xo = x1 + y
            xres_ref[pl.ds(row, TS), :] = xo
            ostage_ref[pl.ds(row, TS), :] = xo.astype(_BF)

            @pl.when(li == 1)
            def _():
                pltpu.make_async_copy(ostage_ref.at[pl.ds(row, TS), :], o_hbm.at[pl.ds(row, TS), :],
                                      out_sems.at[t]).start()
            return c

        lax.fori_loop(0, NT, phase2, 0)
        return carry

    lax.fori_loop(0, 2, layer, 0)

    for t in range(NT):
        pltpu.make_async_copy(ostage_ref.at[t * TS:(t + 1) * TS, :], o_hbm.at[t * TS:(t + 1) * TS, :],
                              out_sems.at[t]).wait()


@jax.jit
def pallas_interleave_layers__linear_kernel_hedgehog__dense_activation_silu__prompt_kernel(
    A_x: jax.Array,
    A_wqkv: jax.Array,
    A_w_phi: jax.Array,
    A_wo: jax.Array,
    B_x: jax.Array,
    B_w1: jax.Array,
    B_w2: jax.Array,
):
    del B_x
    x2 = A_x.reshape(S, D)
    wphi2d = A_w_phi.reshape(H * DH, DH)
    w1t = B_w1.T

    any_spec = pl.BlockSpec(memory_space=pl.ANY)
    out = pl.pallas_call(
        _kernel,
        out_shape=jax.ShapeDtypeStruct((S, D), A_x.dtype),
        in_specs=[any_spec] * 6,
        out_specs=any_spec,
        scratch_shapes=[
            pltpu.VMEM((S, D), _BF),
            pltpu.VMEM((D, 3 * D), _BF),
            pltpu.VMEM((H * DH, DH), _BF),
            pltpu.VMEM((D, D), _BF),
            pltpu.VMEM((FF, D), _BF),
            pltpu.VMEM((FF, D), _BF),
            pltpu.VMEM((S, D), _BF),
            pltpu.VMEM((S, D), _F32),
            pltpu.VMEM((S, D), _BF),
            pltpu.VMEM((3 * D, D), _BF),
            pltpu.VMEM((NG, GR, 2 * GR), _F32),
            pltpu.VMEM((NG, 2 * GR, 128), _F32),
            pltpu.VMEM((NG, GR, 2 * GR), _BF),
            pltpu.VMEM((NG, 2 * GR, 128), _F32),
            pltpu.SemaphoreType.DMA((7,)),
            pltpu.SemaphoreType.DMA((NT,)),
            pltpu.SemaphoreType.DMA((NT,)),
        ],
        compiler_params=pltpu.CompilerParams(vmem_limit_bytes=96 * 1024 * 1024),
    )(x2, A_wqkv, wphi2d, A_wo, w1t, B_w2)
    return out.reshape(1, S, D)
```

```python
import jax
import jax.numpy as jnp
from jax import lax
import jax.experimental.pallas as pl
import jax.experimental.pallas.tpu as pltpu

S = 2048
D = 640
H = 32
DH = 20
FF = 1728
HG = 2
LG = 1
NG = H // HG
GR = HG * DH
NV = GR // 8
TS = 512
NT = S // TS
LOG2E = 1.4426950408889634

_BF = jnp.bfloat16
_F32 = jnp.float32


def _dot_nn(a, b):
    return lax.dot_general(a, b, (((1,), (0,)), ((), ())), preferred_element_type=_F32)


def _dot_nt(a, b):
    return lax.dot_general(a, b, (((1,), (1,)), ((), ())), preferred_element_type=_F32)


def _dot_tn(a, b):
    return lax.dot_general(a, b, (((0,), (0,)), ((), ())), preferred_element_type=_F32)


def _ln_stats(x):
    m = jnp.mean(x, axis=-1, keepdims=True)
    xc = x - m
    v = jnp.mean(xc * xc, axis=-1, keepdims=True)
    return m, xc, v


def _layernorm(x):
    _, xc, v = _ln_stats(x)
    return xc / jnp.sqrt(v + 1e-5)


def _head_reduce(x, op, op2):
    r = op(x, axis=0)
    r = op2(r, pltpu.roll(r, 4, 0))
    r = op2(pltpu.roll(r, 2, 0), r)
    return r[None]


def _head_sum(x):
    return _head_reduce(x, jnp.sum, jnp.add)


def _exps(p):
    mx = _head_reduce(p, jnp.max, jnp.maximum)
    mn = _head_reduce(p, jnp.min, jnp.minimum)
    ea = jnp.exp2(p - mx)
    eb = jnp.exp2(mn - p)
    return ea, eb, _head_sum(ea), _head_sum(eb)


def _kernel(x_hbm, wqkv_hbm, wphi_hbm, wo_hbm, w1t_hbm, w2_hbm, o_hbm,
            x_ref, wqkv_ref, wphi_ref, wo_ref, w1t_ref, w2_ref, ostage_ref,
            xres_ref, xn_ref, wallt_ref, kv_ref, z_ref, kvb_ref, zc_ref, cw_ref,
            in_sems, out_sems, x_sems):
    cp_phi = pltpu.make_async_copy(wphi_hbm, wphi_ref, in_sems.at[0])
    cp_wq = pltpu.make_async_copy(wqkv_hbm.at[:, 0:D], wqkv_ref.at[:, 0:D], in_sems.at[1])
    cp_wk = pltpu.make_async_copy(wqkv_hbm.at[:, D:2 * D], wqkv_ref.at[:, D:2 * D], in_sems.at[2])
    cp_wv = pltpu.make_async_copy(wqkv_hbm.at[:, 2 * D:3 * D], wqkv_ref.at[:, 2 * D:3 * D], in_sems.at[3])
    cp_x = [pltpu.make_async_copy(x_hbm.at[t * TS:(t + 1) * TS, :], x_ref.at[t * TS:(t + 1) * TS, :],
                                  x_sems.at[t]) for t in range(NT)]
    cp_wo = pltpu.make_async_copy(wo_hbm, wo_ref, in_sems.at[4])
    cp_w1 = pltpu.make_async_copy(w1t_hbm, w1t_ref, in_sems.at[5])
    cp_w2 = pltpu.make_async_copy(w2_hbm, w2_ref, in_sems.at[6])
    for cp in [cp_phi, cp_wq, cp_wk, cp_wv] + cp_x + [cp_wo, cp_w1, cp_w2]:
        cp.start()

    g3 = lax.broadcasted_iota(jnp.int32, (NG, GR, D), 0)
    r3 = lax.broadcasted_iota(jnp.int32, (NG, GR, D), 1)
    c3 = lax.broadcasted_iota(jnp.int32, (NG, GR, D), 2)
    hh = g3 * HG + (r3 & (HG - 1))
    amask = ((c3 >= hh * DH) & (c3 < hh * DH + DH)).reshape(D, D)
    rs = lax.broadcasted_iota(jnp.int32, (NG, GR, DH), 1)
    fs = lax.broadcasted_iota(jnp.int32, (NG, GR, DH), 2)
    sel = ((rs >> LG) == fs).astype(_BF).reshape(D, DH)
    kr = lax.broadcasted_iota(jnp.int32, (GR, 2 * GR), 0)
    kc = lax.broadcasted_iota(jnp.int32, (GR, 2 * GR), 1)
    jj = kc & (HG - 1)
    kvmask = (kr >= jj * DH) & (kr < jj * DH + DH)

    cp_phi.wait()
    a_dense = jnp.where(amask, _dot_nt(sel, wphi_ref[...]), 0.0)
    cp_wq.wait()
    for b in range(4):
        lo = (160 * b // 128) * 128
        blk = a_dense[160 * b:160 * (b + 1), lo:lo + 256].astype(_BF)
        wallt_ref[160 * b:160 * (b + 1), :] = (
            _dot_nt(blk, wqkv_ref[:, lo:lo + 256]) * LOG2E).astype(_BF)
    cp_wk.wait()
    for b in range(4):
        lo = (160 * b // 128) * 128
        blk = a_dense[160 * b:160 * (b + 1), lo:lo + 256].astype(_BF)
        wallt_ref[D + 160 * b:D + 160 * (b + 1), :] = (
            _dot_nt(blk, wqkv_ref[:, D + lo:D + lo + 256]) * LOG2E).astype(_BF)
    cp_wv.wait()
    wallt_ref[2 * D:3 * D, :] = wqkv_ref[:, 2 * D:3 * D].T

    def layer(li, carry):
        kv_ref[...] = jnp.zeros(kv_ref.shape, _F32)
        z_ref[...] = jnp.zeros(z_ref.shape, _F32)

        def phase1(t, c):
            row = pl.multiple_of(t * TS, TS)

            @pl.when(li == 0)
            def _():
                pltpu.make_async_copy(x_hbm.at[pl.ds(row, TS), :], x_ref.at[pl.ds(row, TS), :],
                                      x_sems.at[t]).wait()
                xres_ref[pl.ds(row, TS), :] = x_ref[pl.ds(row, TS), :].astype(_F32)

            xn = _layernorm(xres_ref[pl.ds(row, TS), :]).astype(_BF)
            xn_ref[pl.ds(row, TS), :] = xn
            pt = _dot_nt(wallt_ref[D:3 * D, :], xn)
            for gi in range(NG):
                ea, eb, sa, sb = _exps(pt[gi * GR:(gi + 1) * GR].reshape(NV, 8, TS))
                q = 1.0 / (sa * sb)
                phi = jnp.concatenate([(ea * (sb * q)).reshape(GR, TS),
                                       (eb * (sa * q)).reshape(GR, TS)], axis=0)
                vt = pt[D + gi * GR:D + (gi + 1) * GR].astype(_BF)
                kv_ref[gi] += _dot_nt(vt, phi.astype(_BF))
                zp = phi[:, 0:128]
                for i in range(1, TS // 128):
                    zp = zp + phi[:, i * 128:(i + 1) * 128]
                z_ref[gi] += zp
            return c

        lax.fori_loop(0, NT, phase1, 0)

        for gi in range(NG):
            kvb_ref[gi] = jnp.where(kvmask, kv_ref[gi], 0.0).astype(_BF)
            zc = jnp.sum(z_ref[gi], axis=1, keepdims=True)
            zc_ref[gi] = jnp.broadcast_to(zc, (2 * GR, 128))

        @pl.when(li == 0)
        def _():
            cp_wo.wait()
            cp_w1.wait()
            cp_w2.wait()
            cw_ref[...] = _dot_nt(jnp.ones((8, D), _BF), w1t_ref[...])

        def phase2(t, c):
            row = pl.multiple_of(t * TS, TS)
            pq = _dot_nt(wallt_ref[0:D, :], xn_ref[pl.ds(row, TS), :])
            ots = []
            for gi in range(NG):
                ea, eb, sa, sb = _exps(pq[gi * GR:(gi + 1) * GR].reshape(NV, 8, TS))
                zc = zc_ref[gi][:, 0:1]
                za = zc[0:GR].reshape(NV, 8, 1)
                zb = zc[GR:2 * GR].reshape(NV, 8, 1)
                q = 1.0 / (_head_sum(ea * za) * sb + _head_sum(eb * zb) * sa + 1e-6 * (sa * sb))
                phi = jnp.concatenate([(ea * (sb * q)).reshape(GR, TS),
                                       (eb * (sa * q)).reshape(GR, TS)], axis=0)
                ots.append(_dot_nn(kvb_ref[gi], phi.astype(_BF)))
            ot = jnp.concatenate(ots, axis=0).astype(_BF)
            att = _dot_tn(ot, wo_ref[...])
            x1 = xres_ref[pl.ds(row, TS), :] + att
            m, _, v = _ln_stats(x1)
            r = 1.0 / jnp.sqrt(v + 1e-5)
            raw = _dot_nt(x1.astype(_BF), w1t_ref[...])
            h = raw * r - (m * r) * cw_ref[0:1, :]
            h = h * (0.5 + 0.5 * jnp.tanh(0.5 * h))
            y = _dot_nn(h.astype(_BF), w2_ref[...])
            xo = x1 + y
            xres_ref[pl.ds(row, TS), :] = xo
            ostage_ref[pl.ds(row, TS), :] = xo.astype(_BF)

            @pl.when(li == 1)
            def _():
                pltpu.make_async_copy(ostage_ref.at[pl.ds(row, TS), :], o_hbm.at[pl.ds(row, TS), :],
                                      out_sems.at[t]).start()
            return c

        lax.fori_loop(0, NT, phase2, 0)
        return carry

    lax.fori_loop(0, 2, layer, 0)

    for t in range(NT):
        pltpu.make_async_copy(ostage_ref.at[t * TS:(t + 1) * TS, :], o_hbm.at[t * TS:(t + 1) * TS, :],
                              out_sems.at[t]).wait()


@jax.jit
def pallas_interleave_layers__linear_kernel_hedgehog__dense_activation_silu__prompt_kernel(
    A_x: jax.Array,
    A_wqkv: jax.Array,
    A_w_phi: jax.Array,
    A_wo: jax.Array,
    B_x: jax.Array,
    B_w1: jax.Array,
    B_w2: jax.Array,
):
    del B_x
    x2 = A_x.reshape(S, D)
    wphi2d = A_w_phi.reshape(H * DH, DH)
    w1t = B_w1.T

    any_spec = pl.BlockSpec(memory_space=pl.ANY)
    out = pl.pallas_call(
        _kernel,
        out_shape=jax.ShapeDtypeStruct((S, D), A_x.dtype),
        in_specs=[any_spec] * 6,
        out_specs=any_spec,
        scratch_shapes=[
            pltpu.VMEM((S, D), _BF),
            pltpu.VMEM((D, 3 * D), _BF),
            pltpu.VMEM((H * DH, DH), _BF),
            pltpu.VMEM((D, D), _BF),
            pltpu.VMEM((FF, D), _BF),
            pltpu.VMEM((FF, D), _BF),
            pltpu.VMEM((S, D), _BF),
            pltpu.VMEM((S, D), _F32),
            pltpu.VMEM((S, D), _BF),
            pltpu.VMEM((3 * D, D), _BF),
            pltpu.VMEM((NG, GR, 2 * GR), _F32),
            pltpu.VMEM((NG, 2 * GR, 128), _F32),
            pltpu.VMEM((NG, GR, 2 * GR), _BF),
            pltpu.VMEM((NG, 2 * GR, 128), _F32),
            pltpu.VMEM((8, FF), _F32),
            pltpu.SemaphoreType.DMA((7,)),
            pltpu.SemaphoreType.DMA((NT,)),
            pltpu.SemaphoreType.DMA((NT,)),
        ],
        compiler_params=pltpu.CompilerParams(vmem_limit_bytes=96 * 1024 * 1024),
    )(x2, A_wqkv, wphi2d, A_wo, w1t, B_w2)
    return out.reshape(1, S, D)
```
